```python
import os as _os
_os.environ.setdefault("JAX_PLATFORMS", "cpu")
import jax
import jax.numpy as jnp

def _softmax(x, axis=-1):
    return jax.nn.softmax(x, axis=axis)
def _gelu(x):
    return jax.nn.gelu(x, approximate=True)
def _silu(x):
    return jax.nn.silu(x)
def _sigmoid(x):
    return jax.nn.sigmoid(x)
def _layernorm(x, axis=-1, eps=1e-5):
    m = jnp.mean(x, axis=axis, keepdims=True)
    v = jnp.var(x, axis=axis, keepdims=True)
    return (x - m) / jnp.sqrt(v + eps)
def _scatter_add(tgt, idx, src, axis=0):
    return tgt.at[idx].add(src)
def _segment_sum(src, seg, n):
    return jax.ops.segment_sum(src, seg, n)
class _Rng:
    def __init__(self, key):
        self._k = key
    def _next(self):
        self._k, sub = jax.random.split(self._k)
        return sub
    def normal(self, shape):
        return jax.random.normal(self._next(), shape, dtype=jnp.bfloat16)
    def randint(self, lo, hi, shape):
        return jax.random.randint(self._next(), shape, lo, hi, dtype=jnp.int32)
    def uniform(self, shape, lo=0.0, hi=1.0):
        return jax.random.uniform(self._next(), shape, jnp.bfloat16, lo, hi)
    def permutation(self, n):
        return jax.random.permutation(self._next(), n)


kernel_name = 'sequential_preLN__mha_block__dense_activation_mish__prompt'

def setup_inputs():
    _rng = _Rng(jax.random.key(int.from_bytes(__import__("os").urandom(4), "little")))
    _w = (lambda a: (lambda t: t.astype(jnp.bfloat16) if jnp.issubdtype(t.dtype, jnp.floating) else t)(jnp.asarray(a)))
    def _A_setup():
        B, S, D, H = 1, 2048, 576, 32
        return {
            "x": _w((lambda *s: _rng.normal(s) * 0.05)(B, S, D)),
            "wqkv": _w((lambda *s: _rng.normal(s) * 0.05)(D, 3 * D)),
            "wo": _w((lambda *s: _rng.normal(s) * 0.05)(D, D)),
        }
    _A_in = _A_setup()

    def _B_setup():
        B, S, D, F = 1, 2048, 576, 4608
        return {
            "x": _w((lambda *s: _rng.normal(s) * 0.05)(B, S, D)),
            "w1": _w((lambda *s: _rng.normal(s) * 1.6)(D, F) * (D ** -0.5)),
            "b1": _w((lambda *s: _rng.normal(s) * 0.05)(F)),
            "w2": _w((lambda *s: _rng.normal(s) * 0.05)(F, D) * (F ** -0.5)),
        }
    _B_in = _B_setup()

    return {
        "A_x": _A_in["x"],
        "A_wqkv": _A_in["wqkv"],
        "A_wo": _A_in["wo"],
        "B_x": _B_in["x"],
        "B_w1": _B_in["w1"],
        "B_b1": _B_in["b1"],
        "B_w2": _B_in["w2"],
    }

def reference(A_x, A_wqkv, A_wo, B_x, B_w1, B_b1, B_w2):
    def _A_ref(x, wqkv, wo):
        B, S, D = x.shape
        H = 32
        Dh = D // H
        qkv = (lambda x, *d: x.transpose(*d))((x @ wqkv).reshape(B, S, 3, H, Dh), 2, 0, 3, 1, 4)
        q, k, v = qkv[0], qkv[1], qkv[2]
        scores = jnp.einsum("bhqd,bhkd->bhqk", q, k) * (Dh ** -0.5)
        p = _softmax(scores, axis=-1)
        o = jnp.einsum("bhqk,bhkd->bhqd", p, v)
        return (lambda x, *d: x.transpose(*d))(o, 0, 2, 1, 3).reshape(B, S, D) @ wo

    def _B_ref(x, w1, b1, w2):
        h = jnp.einsum("bsd,df->bsf", x, w1) + b1
        sp = jnp.log1p(jnp.exp(-jnp.abs(h))) + jnp.where(h > 0, h, jnp.zeros_like(h))
        act = h * jnp.tanh(sp)
        return jnp.einsum("bsf,fd->bsd", act, w2)

    x = A_x
    h = x + _A_ref(_layernorm(x, axis=-1), A_wqkv, A_wo)
    h2 = h + _B_ref(_layernorm(h, axis=-1), B_w1, B_b1, B_w2)
    return h2
```

```python
import functools
import math

import jax
import jax.numpy as jnp
import jax.experimental.pallas as pl
import jax.experimental.pallas.tpu as pltpu

H = 32
HPG = 7
LANES = 128
EPS = 1e-5


def _layernorm_f32(x):
    m = jnp.mean(x, axis=-1, keepdims=True)
    xc = x - m
    v = jnp.mean(xc * xc, axis=-1, keepdims=True)
    return xc * jax.lax.rsqrt(v + EPS)


def _kernel(x_ref, wqkv_ref, wo_ref, w1_ref, b1_ref, w2_ref, o_ref,
            kt_ref, vm_ref, q_ref, oacc_ref,
            *, seq, dh, groups, tq, f_chunk, kv_chunk):
    f32 = jnp.float32
    bf16 = jnp.bfloat16
    gw = groups * LANES
    i = pl.program_id(0)

    @pl.when(i == 0)
    def _():
        lane = jax.lax.broadcasted_iota(jnp.int32, (kv_chunk, LANES), 1)
        for c in range(seq // kv_chunk):
            rows = pl.ds(c * kv_chunk, kv_chunk)
            ln = _layernorm_f32(x_ref[rows, :].astype(f32)).astype(bf16)
            kv = jnp.dot(ln, wqkv_ref[:, gw:3 * gw], preferred_element_type=f32)
            for g in range(groups):
                kt_ref[g, :, rows] = kv[:, g * LANES:(g + 1) * LANES].T.astype(bf16)
            for h in range(H):
                g, hh = divmod(h, HPG)
                vg = kv[:, gw + g * LANES: gw + (g + 1) * LANES]
                ones_col = jnp.where(lane == LANES - 1, 1.0, 0.0)
                vm = jnp.where((lane >= hh * dh) & (lane < (hh + 1) * dh), vg, ones_col)
                vm_ref[h, rows, :] = vm.astype(bf16)

    xb = x_ref[pl.ds(pl.multiple_of(i * tq, tq), tq), :].astype(f32)
    ln = _layernorm_f32(xb).astype(bf16)
    qscale = (dh ** -0.5) * math.log2(math.e)
    q = jnp.dot(ln, wqkv_ref[:, 0:gw], preferred_element_type=f32) * qscale
    for g in range(groups):
        q_ref[g] = q[:, g * LANES:(g + 1) * LANES].astype(bf16)
    oacc_ref[...] = jnp.zeros(oacc_ref.shape, f32)

    lane_q = jax.lax.broadcasted_iota(jnp.int32, (tq, LANES), 1)

    def head_body(h, carry):
        g = h // HPG
        hh = h % HPG
        qg = q_ref[g]
        lo = hh * dh
        qm = jnp.where((lane_q >= lo) & (lane_q < lo + dh), qg, jnp.zeros_like(qg))
        s = jnp.dot(qm, kt_ref[g], preferred_element_type=f32)
        m = jnp.max(s, axis=1, keepdims=True)
        p = jnp.exp2(s - m).astype(bf16)
        o = jnp.dot(p, vm_ref[h], preferred_element_type=f32)
        inv_l = 1.0 / o[:, LANES - 1:LANES]
        oacc_ref[g] += o * inv_l
        return carry

    jax.lax.fori_loop(0, H, head_body, 0)

    attn = jnp.concatenate([oacc_ref[g].astype(bf16) for g in range(groups)], axis=1)
    h1 = xb + jnp.dot(attn, wo_ref[...], preferred_element_type=f32)

    ln2 = _layernorm_f32(h1).astype(bf16)
    ff = w1_ref.shape[1]
    acc = h1
    for c in range(ff // f_chunk):
        cols = slice(c * f_chunk, (c + 1) * f_chunk)
        z = jnp.dot(ln2, w1_ref[:, cols], preferred_element_type=f32) + b1_ref[:, cols].astype(f32)
        sp = jnp.log1p(jnp.exp(-jnp.abs(z))) + jnp.maximum(z, 0.0)
        act = (z * jnp.tanh(sp)).astype(bf16)
        acc = acc + jnp.dot(act, w2_ref[cols, :], preferred_element_type=f32)
    o_ref[...] = acc.astype(o_ref.dtype)


@jax.jit
def pallas_sequential_preLN__mha_block__dense_activation_mish__prompt_kernel(
    A_x: jax.Array,
    A_wqkv: jax.Array,
    A_wo: jax.Array,
    B_x: jax.Array,
    B_w1: jax.Array,
    B_b1: jax.Array,
    B_w2: jax.Array,
):
    b, seq, d = A_x.shape
    assert b == 1
    dh = d // H
    groups = -(-H // HPG)
    gw = groups * LANES
    ff = B_w1.shape[1]
    tq = 256

    pad_h = groups * HPG - H
    w = A_wqkv.reshape(d, 3, H, dh)
    w = jnp.pad(w, ((0, 0), (0, 0), (0, pad_h), (0, 0)))
    w = w.reshape(d, 3, groups, HPG * dh)
    w = jnp.pad(w, ((0, 0), (0, 0), (0, 0), (0, LANES - HPG * dh)))
    wqkv_p = w.reshape(d, 3 * gw)

    w = A_wo.reshape(H, dh, d)
    w = jnp.pad(w, ((0, pad_h), (0, 0), (0, 0)))
    w = w.reshape(groups, HPG * dh, d)
    w = jnp.pad(w, ((0, 0), (0, LANES - HPG * dh), (0, 0)))
    wo_p = w.reshape(gw, d)

    x2 = A_x.reshape(seq, d)
    b1 = B_b1.reshape(1, ff)

    kern = functools.partial(_kernel, seq=seq, dh=dh, groups=groups, tq=tq,
                             f_chunk=512, kv_chunk=512)
    const = lambda i: (0, 0)
    out = pl.pallas_call(
        kern,
        grid=(seq // tq,),
        in_specs=[
            pl.BlockSpec((seq, d), const),
            pl.BlockSpec((d, 3 * gw), const),
            pl.BlockSpec((gw, d), const),
            pl.BlockSpec((d, ff), const),
            pl.BlockSpec((1, ff), const),
            pl.BlockSpec((ff, d), const),
        ],
        out_specs=pl.BlockSpec((tq, d), lambda i: (i, 0)),
        out_shape=jax.ShapeDtypeStruct((seq, d), A_x.dtype),
        scratch_shapes=[
            pltpu.VMEM((groups, LANES, seq), jnp.bfloat16),
            pltpu.VMEM((H, seq, LANES), jnp.bfloat16),
            pltpu.VMEM((groups, tq, LANES), jnp.bfloat16),
            pltpu.VMEM((groups, tq, LANES), jnp.float32),
        ],
        compiler_params=pltpu.CompilerParams(
            dimension_semantics=("arbitrary",),
            vmem_limit_bytes=100 * 1024 * 1024,
        ),
    )(x2, wqkv_p, wo_p, B_w1, b1, B_w2)
    return out.reshape(b, seq, d)
```

```python
import functools
import math

import jax
import jax.numpy as jnp
import jax.experimental.pallas as pl
import jax.experimental.pallas.tpu as pltpu

H = 32
HPG = 7
LANES = 128
EPS = 1e-5
VROWS = 32
OROWS = 24


def _layernorm_t(xt):
    m = jnp.mean(xt, axis=0, keepdims=True)
    xc = xt - m
    v = jnp.mean(xc * xc, axis=0, keepdims=True)
    return xc * jax.lax.rsqrt(v + EPS)


def _kernel(xt_ref, b1_ref, wqkv_hbm, wo_hbm, w1_hbm, w2t_hbm, o_ref,
            wqkv_raw, wo_raw, w1_raw, w2t_ref, wt_ref, wot_ref, w1t_ref,
            qt_ref, k_ref, vt_ref, ot_ref, a2_ref, acc_ref,
            sa_ref, sb_ref, ma_ref, mb_ref, sems,
            *, seq, d, dh, groups, tq, f_chunk, kv_chunk):
    f32 = jnp.float32
    bf16 = jnp.bfloat16
    gw = groups * LANES
    gh = HPG * dh
    dk = a2_ref.shape[0]
    ff = w1t_ref.shape[0]
    i = pl.program_id(0)

    copies = [
        pltpu.make_async_copy(wqkv_hbm, wqkv_raw, sems.at[0]),
        pltpu.make_async_copy(wo_hbm, wo_raw, sems.at[1]),
        pltpu.make_async_copy(w1_hbm, w1_raw, sems.at[2]),
        pltpu.make_async_copy(w2t_hbm, w2t_ref, sems.at[3]),
    ]

    @pl.when(i == 0)
    def _():
        for cp in copies:
            cp.start()
        copies[0].wait()
        wt_ref[...] = jnp.zeros(wt_ref.shape, bf16)
        wraw_t = wqkv_raw[...].astype(f32).T
        for t in range(2):
            for g in range(groups):
                w = min(gh, d - g * gh)
                wt_ref[t * gw + g * LANES: t * gw + g * LANES + w, :] = (
                    wraw_t[t * d + g * gh: t * d + g * gh + w, :].astype(bf16))
        wt_ref[2 * gw: 2 * gw + d, :] = wraw_t[2 * d: 3 * d, :].astype(bf16)

        qscale = (dh ** -0.5) * math.log2(math.e)
        pad_rows = jnp.concatenate(
            [jnp.ones((1, kv_chunk), f32), jnp.zeros((VROWS - dh - 1, kv_chunk), f32)], axis=0)

        def qkv_chunk(c, carry):
            cols = pl.ds(pl.multiple_of(c * kv_chunk, kv_chunk), kv_chunk)
            ln = _layernorm_t(xt_ref[:, cols].astype(f32)).astype(bf16)
            qkv = jnp.dot(wt_ref[...], ln, preferred_element_type=f32)
            qt_ref[:, cols] = (qkv[0:gw] * qscale).astype(bf16)
            for g in range(groups):
                k_ref[g, cols, :] = qkv[gw + g * LANES: gw + (g + 1) * LANES].T.astype(bf16)
            for h in range(H):
                vh = qkv[2 * gw + h * dh: 2 * gw + (h + 1) * dh]
                vt_ref[h, :, cols] = jnp.concatenate([vh, pad_rows], axis=0).astype(bf16)
            return carry

        jax.lax.fori_loop(0, seq // kv_chunk, qkv_chunk, 0)

        copies[1].wait()
        wo_f = wo_raw[...].astype(f32)
        parts = []
        for h in range(H):
            parts.append(wo_f[h * dh:(h + 1) * dh, :])
            parts.append(jnp.zeros((OROWS - dh, d), f32))
        wot_ref[...] = jnp.concatenate(parts, axis=0).T.astype(bf16)

        copies[2].wait()

        def w1_chunk(c, carry):
            cols = pl.ds(pl.multiple_of(c * f_chunk, f_chunk), f_chunk)
            aug = jnp.concatenate(
                [w1_raw[:, cols].astype(f32), b1_ref[:, cols].astype(f32),
                 jnp.zeros((dk - d - 1, f_chunk), f32)], axis=0)
            w1t_ref[cols, :] = aug.T.astype(bf16)
            return carry

        jax.lax.fori_loop(0, ff // f_chunk, w1_chunk, 0)
        copies[3].wait()

    qcols = pl.ds(pl.multiple_of(i * tq, tq), tq)
    row_q = jax.lax.broadcasted_iota(jnp.int32, (LANES, tq), 0)

    def scores(h, s_ref, m_ref):
        g = h // HPG
        hh = h % HPG
        qg = qt_ref[pl.ds(pl.multiple_of(g * LANES, LANES), LANES), qcols]
        lo = hh * dh
        qm = jnp.where((row_q >= lo) & (row_q < lo + dh), qg, jnp.zeros_like(qg))
        s = jnp.dot(k_ref[g], qm, preferred_element_type=f32)
        s_ref[...] = s
        m_ref[...] = jnp.max(s, axis=0, keepdims=True)

    def finish(h, s_ref, m_ref):
        p = jnp.exp2(s_ref[...] - m_ref[...]).astype(bf16)
        o = jnp.dot(vt_ref[h], p, preferred_element_type=f32)
        ot_ref[h] = o[0:OROWS] * (1.0 / o[dh:dh + 1])

    scores(0, sa_ref, ma_ref)

    def pair_body(j, carry):
        h = 2 * j
        scores(h + 1, sb_ref, mb_ref)
        finish(h, sa_ref, ma_ref)
        scores(jnp.minimum(h + 2, H - 1), sa_ref, ma_ref)
        finish(h + 1, sb_ref, mb_ref)
        return carry

    jax.lax.fori_loop(0, H // 2, pair_body, 0)

    xb = xt_ref[:, qcols].astype(f32)
    attn = ot_ref[...].reshape(H * OROWS, tq).astype(bf16)
    h1 = xb + jnp.dot(wot_ref[...], attn, preferred_element_type=f32)

    a2_ref[0:d, :] = _layernorm_t(h1).astype(bf16)
    a2_ref[d:dk, :] = jnp.where(
        jax.lax.broadcasted_iota(jnp.int32, (dk - d, tq), 0) == 0, 1.0, 0.0).astype(bf16)
    acc_ref[...] = h1

    def mlp_chunk(c, carry):
        rows = pl.ds(pl.multiple_of(c * f_chunk, f_chunk), f_chunk)
        z = jnp.dot(w1t_ref[rows, :], a2_ref[...], preferred_element_type=f32)
        sp = jnp.log1p(jnp.exp(-jnp.abs(z))) + jnp.maximum(z, 0.0)
        act = (z * jnp.tanh(sp)).astype(bf16)
        acc_ref[...] += jnp.dot(w2t_ref[:, rows], act, preferred_element_type=f32)
        return carry

    jax.lax.fori_loop(0, ff // f_chunk, mlp_chunk, 0)
    o_ref[...] = acc_ref[...].astype(o_ref.dtype)


@jax.jit
def pallas_sequential_preLN__mha_block__dense_activation_mish__prompt_kernel(
    A_x: jax.Array,
    A_wqkv: jax.Array,
    A_wo: jax.Array,
    B_x: jax.Array,
    B_w1: jax.Array,
    B_b1: jax.Array,
    B_w2: jax.Array,
):
    b, seq, d = A_x.shape
    assert b == 1
    dh = d // H
    groups = -(-H // HPG)
    gw = groups * LANES
    ff = B_w1.shape[1]
    dk = -(-(d + 1) // LANES) * LANES
    tq = 256

    xt = A_x.reshape(seq, d).T
    b1 = B_b1.reshape(1, ff)
    w2t = B_w2.T

    kern = functools.partial(_kernel, seq=seq, d=d, dh=dh, groups=groups, tq=tq,
                             f_chunk=512, kv_chunk=512)
    const = lambda i: (0, 0)
    bf16 = jnp.bfloat16
    f32 = jnp.float32
    out_t = pl.pallas_call(
        kern,
        grid=(seq // tq,),
        in_specs=[
            pl.BlockSpec((d, seq), const),
            pl.BlockSpec((1, ff), const),
            pl.BlockSpec(memory_space=pl.ANY),
            pl.BlockSpec(memory_space=pl.ANY),
            pl.BlockSpec(memory_space=pl.ANY),
            pl.BlockSpec(memory_space=pl.ANY),
        ],
        out_specs=pl.BlockSpec((d, tq), lambda i: (0, i)),
        out_shape=jax.ShapeDtypeStruct((d, seq), A_x.dtype),
        scratch_shapes=[
            pltpu.VMEM((d, 3 * d), bf16),
            pltpu.VMEM((d, d), bf16),
            pltpu.VMEM((d, ff), bf16),
            pltpu.VMEM((d, ff), bf16),
            pltpu.VMEM((2 * gw + d, d), bf16),
            pltpu.VMEM((d, H * OROWS), bf16),
            pltpu.VMEM((ff, dk), bf16),
            pltpu.VMEM((gw, seq), bf16),
            pltpu.VMEM((groups, seq, LANES), bf16),
            pltpu.VMEM((H, VROWS, seq), bf16),
            pltpu.VMEM((H, OROWS, tq), f32),
            pltpu.VMEM((dk, tq), bf16),
            pltpu.VMEM((d, tq), f32),
            pltpu.VMEM((seq, tq), f32),
            pltpu.VMEM((seq, tq), f32),
            pltpu.VMEM((1, tq), f32),
            pltpu.VMEM((1, tq), f32),
            pltpu.SemaphoreType.DMA((4,)),
        ],
        compiler_params=pltpu.CompilerParams(
            dimension_semantics=("arbitrary",),
            vmem_limit_bytes=100 * 1024 * 1024,
        ),
    )(xt, b1, A_wqkv, A_wo, B_w1, w2t)
    return out_t.T.reshape(b, seq, d)
```

```python
import functools
import math

import jax
import jax.numpy as jnp
import jax.experimental.pallas as pl
import jax.experimental.pallas.tpu as pltpu

H = 32
HPG = 7
LANES = 128
EPS = 1e-5
VROWS = 32
OROWS = 24


def _layernorm_t(xt):
    m = jnp.mean(xt, axis=0, keepdims=True)
    xc = xt - m
    v = jnp.mean(xc * xc, axis=0, keepdims=True)
    return xc * jax.lax.rsqrt(v + EPS)


def _kernel(xt_ref, b1_ref, wqkv_raw, wo_hbm, w1_hbm, w2t_hbm, o_ref,
            wo_raw, w1_raw, w2t_ref, wt_ref, wot_ref, w1t_ref,
            qt_ref, k_ref, vt_ref, ot_ref, a2_ref, acc_ref,
            sa_ref, sb_ref, ma_ref, mb_ref, sems,
            *, seq, d, dh, groups, tq, f_chunk, kv_chunk):
    f32 = jnp.float32
    bf16 = jnp.bfloat16
    gw = groups * LANES
    gh = HPG * dh
    dk = a2_ref.shape[0]
    ff = w1t_ref.shape[0]
    i = pl.program_id(0)

    copies = [
        pltpu.make_async_copy(wo_hbm, wo_raw, sems.at[0]),
        pltpu.make_async_copy(w1_hbm, w1_raw, sems.at[1]),
        pltpu.make_async_copy(w2t_hbm, w2t_ref, sems.at[2]),
    ]

    @pl.when(i == 0)
    def _():
        for cp in copies:
            cp.start()
        wt_ref[...] = jnp.zeros(wt_ref.shape, bf16)
        wraw_t = wqkv_raw[...].astype(f32).T
        for t in range(2):
            for g in range(groups):
                w = min(gh, d - g * gh)
                wt_ref[t * gw + g * LANES: t * gw + g * LANES + w, :] = (
                    wraw_t[t * d + g * gh: t * d + g * gh + w, :].astype(bf16))
        wt_ref[2 * gw: 2 * gw + d, :] = wraw_t[2 * d: 3 * d, :].astype(bf16)

        qscale = (dh ** -0.5) * math.log2(math.e)
        pad_rows = jnp.concatenate(
            [jnp.ones((1, kv_chunk), f32), jnp.zeros((VROWS - dh - 1, kv_chunk), f32)], axis=0)

        def qkv_chunk(c, carry):
            cols = pl.ds(pl.multiple_of(c * kv_chunk, kv_chunk), kv_chunk)
            ln = _layernorm_t(xt_ref[:, cols].astype(f32)).astype(bf16)
            qkv = jnp.dot(wt_ref[...], ln, preferred_element_type=f32)
            qt_ref[:, cols] = (qkv[0:gw] * qscale).astype(bf16)
            for g in range(groups):
                k_ref[g, cols, :] = qkv[gw + g * LANES: gw + (g + 1) * LANES].T.astype(bf16)
            for h in range(H):
                vh = qkv[2 * gw + h * dh: 2 * gw + (h + 1) * dh]
                vt_ref[h, :, cols] = jnp.concatenate([vh, pad_rows], axis=0).astype(bf16)
            return carry

        jax.lax.fori_loop(0, seq // kv_chunk, qkv_chunk, 0)

        copies[0].wait()
        wo_f = wo_raw[...].astype(f32)
        parts = []
        for h in range(H):
            parts.append(wo_f[h * dh:(h + 1) * dh, :])
            parts.append(jnp.zeros((OROWS - dh, d), f32))
        wot_ref[...] = jnp.concatenate(parts, axis=0).T.astype(bf16)

        copies[1].wait()

        def w1_chunk(c, carry):
            cols = pl.ds(pl.multiple_of(c * f_chunk, f_chunk), f_chunk)
            aug = jnp.concatenate(
                [w1_raw[:, cols].astype(f32), b1_ref[:, cols].astype(f32),
                 jnp.zeros((dk - d - 1, f_chunk), f32)], axis=0)
            w1t_ref[cols, :] = aug.T.astype(bf16)
            return carry

        jax.lax.fori_loop(0, ff // f_chunk, w1_chunk, 0)
        copies[2].wait()

    qcols = pl.ds(pl.multiple_of(i * tq, tq), tq)
    row_q = jax.lax.broadcasted_iota(jnp.int32, (LANES, tq), 0)
    nblk = seq // tq

    def scores(h, blk, s_ref, m_ref):
        g = h // HPG
        hh = h % HPG
        qg = qt_ref[pl.ds(pl.multiple_of(g * LANES, LANES), LANES),
                    pl.ds(pl.multiple_of(blk * tq, tq), tq)]
        lo = hh * dh
        qm = jnp.where((row_q >= lo) & (row_q < lo + dh), qg, jnp.zeros_like(qg))
        s = jnp.dot(k_ref[g], qm, preferred_element_type=f32)
        s_ref[...] = s
        m_ref[...] = jnp.max(s, axis=0, keepdims=True)

    def finish(h, s_ref, m_ref):
        p = jnp.exp2(s_ref[...] - m_ref[...]).astype(bf16)
        o = jnp.dot(vt_ref[h], p, preferred_element_type=f32)
        ot_ref[h] = o[0:OROWS] * (1.0 / o[dh:dh + 1])

    @pl.when(i == 0)
    def _():
        scores(0, 0, sa_ref, ma_ref)

    def quad_body(j, carry):
        h = 4 * j
        scores(h + 1, i, sb_ref, mb_ref)
        finish(h, sa_ref, ma_ref)
        scores(h + 2, i, sa_ref, ma_ref)
        finish(h + 1, sb_ref, mb_ref)
        scores(h + 3, i, sb_ref, mb_ref)
        finish(h + 2, sa_ref, ma_ref)
        hn = h + 4
        scores(hn % H, jnp.minimum(i + hn // H, nblk - 1), sa_ref, ma_ref)
        finish(h + 3, sb_ref, mb_ref)
        return carry

    jax.lax.fori_loop(0, H // 4, quad_body, 0)

    xb = xt_ref[:, qcols].astype(f32)
    attn = ot_ref[...].reshape(H * OROWS, tq).astype(bf16)
    h1 = xb + jnp.dot(wot_ref[...], attn, preferred_element_type=f32)

    a2_ref[0:d, :] = _layernorm_t(h1).astype(bf16)
    a2_ref[d:dk, :] = jnp.where(
        jax.lax.broadcasted_iota(jnp.int32, (dk - d, tq), 0) == 0, 1.0, 0.0).astype(bf16)
    acc_ref[...] = h1

    def mlp_chunk(c, carry):
        rows = pl.ds(pl.multiple_of(c * f_chunk, f_chunk), f_chunk)
        z = jnp.dot(w1t_ref[rows, :], a2_ref[...], preferred_element_type=f32)
        sp = jnp.log1p(jnp.exp(-jnp.abs(z))) + jnp.maximum(z, 0.0)
        act = (z * jnp.tanh(sp)).astype(bf16)
        acc_ref[...] += jnp.dot(w2t_ref[:, rows], act, preferred_element_type=f32)
        return carry

    jax.lax.fori_loop(0, ff // f_chunk, mlp_chunk, 0)
    o_ref[...] = acc_ref[...].astype(o_ref.dtype)


@jax.jit
def pallas_sequential_preLN__mha_block__dense_activation_mish__prompt_kernel(
    A_x: jax.Array,
    A_wqkv: jax.Array,
    A_wo: jax.Array,
    B_x: jax.Array,
    B_w1: jax.Array,
    B_b1: jax.Array,
    B_w2: jax.Array,
):
    b, seq, d = A_x.shape
    assert b == 1
    dh = d // H
    groups = -(-H // HPG)
    gw = groups * LANES
    ff = B_w1.shape[1]
    dk = -(-(d + 1) // LANES) * LANES
    tq = 512

    xt = A_x.reshape(seq, d).T
    b1 = B_b1.reshape(1, ff)
    w2t = B_w2.T

    kern = functools.partial(_kernel, seq=seq, d=d, dh=dh, groups=groups, tq=tq,
                             f_chunk=1152, kv_chunk=512)
    const = lambda i: (0, 0)
    bf16 = jnp.bfloat16
    f32 = jnp.float32
    out_t = pl.pallas_call(
        kern,
        grid=(seq // tq,),
        in_specs=[
            pl.BlockSpec((d, seq), const),
            pl.BlockSpec((1, ff), const),
            pl.BlockSpec((d, 3 * d), const),
            pl.BlockSpec(memory_space=pl.ANY),
            pl.BlockSpec(memory_space=pl.ANY),
            pl.BlockSpec(memory_space=pl.ANY),
        ],
        out_specs=pl.BlockSpec((d, tq), lambda i: (0, i)),
        out_shape=jax.ShapeDtypeStruct((d, seq), A_x.dtype),
        scratch_shapes=[
            pltpu.VMEM((d, d), bf16),
            pltpu.VMEM((d, ff), bf16),
            pltpu.VMEM((d, ff), bf16),
            pltpu.VMEM((2 * gw + d, d), bf16),
            pltpu.VMEM((d, H * OROWS), bf16),
            pltpu.VMEM((ff, dk), bf16),
            pltpu.VMEM((gw, seq), bf16),
            pltpu.VMEM((groups, seq, LANES), bf16),
            pltpu.VMEM((H, VROWS, seq), bf16),
            pltpu.VMEM((H, OROWS, tq), f32),
            pltpu.VMEM((dk, tq), bf16),
            pltpu.VMEM((d, tq), f32),
            pltpu.VMEM((seq, tq), f32),
            pltpu.VMEM((seq, tq), f32),
            pltpu.VMEM((1, tq), f32),
            pltpu.VMEM((1, tq), f32),
            pltpu.SemaphoreType.DMA((3,)),
        ],
        compiler_params=pltpu.CompilerParams(
            dimension_semantics=("arbitrary",),
            vmem_limit_bytes=100 * 1024 * 1024,
        ),
    )(xt, b1, A_wqkv, A_wo, B_w1, w2t)
    return out_t.T.reshape(b, seq, d)
```

```python
import functools
import math

import jax
import jax.numpy as jnp
import jax.experimental.pallas as pl
import jax.experimental.pallas.tpu as pltpu

H = 32
HPG = 7
LANES = 128
EPS = 1e-5
VROWS = 32
OROWS = 24


def _layernorm_t(xt):
    m = jnp.mean(xt, axis=0, keepdims=True)
    xc = xt - m
    v = jnp.mean(xc * xc, axis=0, keepdims=True)
    return xc * jax.lax.rsqrt(v + EPS)


def _kernel(xt_ref, b1_ref, wqkv_raw, wo_hbm, w1_hbm, w2t_hbm, o_ref,
            wo_raw, w1_raw, w2t_ref, wt_ref, wot_ref, w1t_ref,
            qt_ref, k_ref, vt_ref, ot_ref, a2_ref, acc_ref,
            sa_ref, sb_ref, ma_ref, mb_ref, sems,
            *, seq, d, dh, groups, tq, f_chunk, kv_chunk):
    f32 = jnp.float32
    bf16 = jnp.bfloat16
    gw = groups * LANES
    gh = HPG * dh
    dk = a2_ref.shape[0]
    ff = w1t_ref.shape[0]
    i = pl.program_id(0)

    copies = [
        pltpu.make_async_copy(wo_hbm, wo_raw, sems.at[0]),
        pltpu.make_async_copy(w1_hbm, w1_raw, sems.at[1]),
        pltpu.make_async_copy(w2t_hbm, w2t_ref, sems.at[2]),
    ]

    @pl.when(i == 0)
    def _():
        for cp in copies:
            cp.start()
        wt_ref[...] = jnp.zeros(wt_ref.shape, bf16)
        wraw_t = wqkv_raw[...].astype(f32).T
        for t in range(2):
            for g in range(groups):
                w = min(gh, d - g * gh)
                wt_ref[t * gw + g * LANES: t * gw + g * LANES + w, :] = (
                    wraw_t[t * d + g * gh: t * d + g * gh + w, :].astype(bf16))
        wt_ref[2 * gw: 2 * gw + d, :] = wraw_t[2 * d: 3 * d, :].astype(bf16)

        qscale = (dh ** -0.5) * math.log2(math.e)
        pad_rows = jnp.concatenate(
            [jnp.ones((1, kv_chunk), f32), jnp.zeros((VROWS - dh - 1, kv_chunk), f32)], axis=0)

        def qkv_chunk(c, carry):
            cols = pl.ds(pl.multiple_of(c * kv_chunk, kv_chunk), kv_chunk)
            ln = _layernorm_t(xt_ref[:, cols].astype(f32)).astype(bf16)
            qkv = jnp.dot(wt_ref[...], ln, preferred_element_type=f32)
            qt_ref[:, cols] = (qkv[0:gw] * qscale).astype(bf16)
            for g in range(groups):
                k_ref[g, cols, :] = qkv[gw + g * LANES: gw + (g + 1) * LANES].T.astype(bf16)
            for h in range(H):
                vh = qkv[2 * gw + h * dh: 2 * gw + (h + 1) * dh]
                vt_ref[h, :, cols] = jnp.concatenate([vh, pad_rows], axis=0).astype(bf16)
            return carry

        jax.lax.fori_loop(0, seq // kv_chunk, qkv_chunk, 0)

        copies[0].wait()
        wo_f = wo_raw[...].astype(f32)
        parts = []
        for h in range(H):
            parts.append(wo_f[h * dh:(h + 1) * dh, :])
            parts.append(jnp.zeros((OROWS - dh, d), f32))
        wot_ref[...] = jnp.concatenate(parts, axis=0).T.astype(bf16)

        copies[1].wait()

        def w1_chunk(c, carry):
            cols = pl.ds(pl.multiple_of(c * f_chunk, f_chunk), f_chunk)
            aug = jnp.concatenate(
                [w1_raw[:, cols].astype(f32), b1_ref[:, cols].astype(f32),
                 jnp.zeros((dk - d - 1, f_chunk), f32)], axis=0)
            w1t_ref[cols, :] = aug.T.astype(bf16)
            return carry

        jax.lax.fori_loop(0, ff // f_chunk, w1_chunk, 0)
        copies[2].wait()

    qcols = pl.ds(pl.multiple_of(i * tq, tq), tq)
    row_q = jax.lax.broadcasted_iota(jnp.int32, (LANES, tq), 0)
    nblk = seq // tq

    def scores(h, blk, s_ref, m_ref):
        g = h // HPG
        hh = h % HPG
        qg = qt_ref[pl.ds(pl.multiple_of(g * LANES, LANES), LANES),
                    pl.ds(pl.multiple_of(blk * tq, tq), tq)]
        lo = hh * dh
        qm = jnp.where((row_q >= lo) & (row_q < lo + dh), qg, jnp.zeros_like(qg))
        s = jnp.dot(k_ref[g], qm, preferred_element_type=f32)
        s_ref[...] = s
        m_ref[...] = jnp.max(s, axis=0, keepdims=True)

    def finish(h, s_ref, m_ref):
        p = jnp.exp2(s_ref[...] - m_ref[...]).astype(bf16)
        o = jnp.dot(vt_ref[h], p, preferred_element_type=f32)
        ot_ref[h] = o[0:OROWS] * (1.0 / o[dh:dh + 1])

    @pl.when(i == 0)
    def _():
        scores(0, 0, sa_ref, ma_ref)

    unroll = 8
    bufs = ((sa_ref, ma_ref), (sb_ref, mb_ref))

    def multi_body(j, carry):
        h = unroll * j
        for u in range(unroll):
            if u + 1 < unroll:
                scores(h + u + 1, i, *bufs[(u + 1) % 2])
            else:
                hn = h + unroll
                scores(hn % H, jnp.minimum(i + hn // H, nblk - 1), *bufs[0])
            finish(h + u, *bufs[u % 2])
        return carry

    jax.lax.fori_loop(0, H // unroll, multi_body, 0)

    xb = xt_ref[:, qcols].astype(f32)
    attn = ot_ref[...].reshape(H * OROWS, tq).astype(bf16)
    h1 = xb + jnp.dot(wot_ref[...], attn, preferred_element_type=f32)

    a2_ref[0:d, :] = _layernorm_t(h1).astype(bf16)
    a2_ref[d:dk, :] = jnp.where(
        jax.lax.broadcasted_iota(jnp.int32, (dk - d, tq), 0) == 0, 1.0, 0.0).astype(bf16)
    acc_ref[...] = h1

    def mlp_chunk(c, carry):
        rows = pl.ds(pl.multiple_of(c * f_chunk, f_chunk), f_chunk)
        z = jnp.dot(w1t_ref[rows, :], a2_ref[...], preferred_element_type=f32)
        sp = jnp.log1p(jnp.exp(-jnp.abs(z))) + jnp.maximum(z, 0.0)
        act = (z * jnp.tanh(sp)).astype(bf16)
        acc_ref[...] += jnp.dot(w2t_ref[:, rows], act, preferred_element_type=f32)
        return carry

    jax.lax.fori_loop(0, ff // f_chunk, mlp_chunk, 0)
    o_ref[...] = acc_ref[...].astype(o_ref.dtype)


@jax.jit
def pallas_sequential_preLN__mha_block__dense_activation_mish__prompt_kernel(
    A_x: jax.Array,
    A_wqkv: jax.Array,
    A_wo: jax.Array,
    B_x: jax.Array,
    B_w1: jax.Array,
    B_b1: jax.Array,
    B_w2: jax.Array,
):
    b, seq, d = A_x.shape
    assert b == 1
    dh = d // H
    groups = -(-H // HPG)
    gw = groups * LANES
    ff = B_w1.shape[1]
    dk = -(-(d + 1) // LANES) * LANES
    tq = 512

    xt = A_x.reshape(seq, d).T
    b1 = B_b1.reshape(1, ff)
    w2t = B_w2.T

    kern = functools.partial(_kernel, seq=seq, d=d, dh=dh, groups=groups, tq=tq,
                             f_chunk=1152, kv_chunk=512)
    const = lambda i: (0, 0)
    bf16 = jnp.bfloat16
    f32 = jnp.float32
    out_t = pl.pallas_call(
        kern,
        grid=(seq // tq,),
        in_specs=[
            pl.BlockSpec((d, seq), const),
            pl.BlockSpec((1, ff), const),
            pl.BlockSpec((d, 3 * d), const),
            pl.BlockSpec(memory_space=pl.ANY),
            pl.BlockSpec(memory_space=pl.ANY),
            pl.BlockSpec(memory_space=pl.ANY),
        ],
        out_specs=pl.BlockSpec((d, tq), lambda i: (0, i)),
        out_shape=jax.ShapeDtypeStruct((d, seq), A_x.dtype),
        scratch_shapes=[
            pltpu.VMEM((d, d), bf16),
            pltpu.VMEM((d, ff), bf16),
            pltpu.VMEM((d, ff), bf16),
            pltpu.VMEM((2 * gw + d, d), bf16),
            pltpu.VMEM((d, H * OROWS), bf16),
            pltpu.VMEM((ff, dk), bf16),
            pltpu.VMEM((gw, seq), bf16),
            pltpu.VMEM((groups, seq, LANES), bf16),
            pltpu.VMEM((H, VROWS, seq), bf16),
            pltpu.VMEM((H, OROWS, tq), f32),
            pltpu.VMEM((dk, tq), bf16),
            pltpu.VMEM((d, tq), f32),
            pltpu.VMEM((seq, tq), f32),
            pltpu.VMEM((seq, tq), f32),
            pltpu.VMEM((1, tq), f32),
            pltpu.VMEM((1, tq), f32),
            pltpu.SemaphoreType.DMA((3,)),
        ],
        compiler_params=pltpu.CompilerParams(
            dimension_semantics=("arbitrary",),
            vmem_limit_bytes=100 * 1024 * 1024,
        ),
    )(xt, b1, A_wqkv, A_wo, B_w1, w2t)
    return out_t.T.reshape(b, seq, d)
```
